```python
import os as _os
_os.environ.setdefault('JAX_PLATFORMS', 'cpu')
import jax
import jax.numpy as jnp

def _softmax(x, axis=-1):
    return jax.nn.softmax(x, axis=axis)

def _gelu(x):
    return jax.nn.gelu(x, approximate=True)

def _silu(x):
    return jax.nn.silu(x)

def _sigmoid(x):
    return jax.nn.sigmoid(x)

def _layernorm(x, axis=-1, eps=1e-05):
    m = jnp.mean(x, axis=axis, keepdims=True)
    v = jnp.var(x, axis=axis, keepdims=True)
    return (x - m) / jnp.sqrt(v + eps)

def _scatter_add(tgt, idx, src, axis=0):
    return tgt.at[idx].add(src)

def _segment_sum(src, seg, n):
    return jax.ops.segment_sum(src, seg, n)

class _Rng:

    def __init__(self, key):
        self._k = key

    def _next(self):
        self._k, sub = jax.random.split(self._k)
        return sub

    def normal(self, shape):
        return jax.random.normal(self._next(), shape, dtype=jnp.bfloat16)

    def randint(self, lo, hi, shape):
        return jax.random.randint(self._next(), shape, lo, hi, dtype=jnp.int32)

    def uniform(self, shape, lo=0.0, hi=1.0):
        return jax.random.uniform(self._next(), shape, jnp.bfloat16, lo, hi)

    def permutation(self, n):
        return jax.random.permutation(self._next(), n)
kernel_name = 'recurrent_scan__spectral_gfnet__mixer_gmlp__prompt'

def setup_inputs():
    _rng = _Rng(jax.random.key(int.from_bytes(__import__("os").urandom(4), "little")))
    _w = lambda a: (lambda t: t.astype(jnp.bfloat16) if jnp.issubdtype(t.dtype, jnp.floating) else t)(jnp.asarray(a))

    def _A_setup():
        B, S, D = (1, 2048, 512)
        Df = D // 2 + 1
        return {'x': _w((lambda *s: _rng.normal(s) * 0.05)(B, S, D)), 'w_r': _w((lambda *s: _rng.normal(s) * 0.1)(S, Df) * 0.02), 'w_i': _w((lambda *s: _rng.normal(s) * 0.1)(S, Df) * 0.02)}
    _A_in = _A_setup()

    def _B_setup():
        B, S, D, F = (1, 2048, 512, 1376)
        Fh = F // 2
        return {'x': _w((lambda *s: _rng.normal(s) * 0.05)(B, S, D)), 'w_in': _w((lambda *s: _rng.normal(s) * 0.4)(D, 2 * Fh)), 'w_sp': _w(0.01 * (lambda *s: _rng.normal(s) * 0.4)(S, S)), 'b_sp': _w(1.0 + 0.01 * (lambda *s: _rng.normal(s) * 0.05)(S)), 'w_out': _w((lambda *s: _rng.normal(s) * 0.05)(Fh, D))}
    _B_in = _B_setup()
    return {'A_x': _A_in['x'], 'A_w_r': _A_in['w_r'], 'A_w_i': _A_in['w_i'], 'B_x': _B_in['x'], 'B_w_in': _B_in['w_in'], 'B_w_sp': _B_in['w_sp'], 'B_b_sp': _B_in['b_sp'], 'B_w_out': _B_in['w_out']}

def reference(A_x, A_w_r, A_w_i, B_x, B_w_in, B_w_sp, B_b_sp, B_w_out):

    def _A_ref(x, w_r, w_i):
        B, S, D = x.shape
        X = (lambda x, axes=(-2, -1): jnp.fft.rfft2(x.astype(jnp.float32), axes=axes))(x, axes=(-2, -1))
        W = w_r + 1j * w_i
        X = X * W
        y = (lambda x, s, axes=(-2, -1): jnp.fft.irfft2(x, s=s, axes=axes).astype(jnp.bfloat16))(X, (S, D), axes=(-2, -1))
        return y

    def _B_ref(x, w_in, w_sp, b_sp, w_out):
        B, S, D = x.shape
        F = w_in.shape[-1]
        Fh = F // 2
        z = _gelu(jnp.einsum('bsd,df->bsf', x, w_in))
        z1 = z[..., :Fh].copy()
        z2 = _layernorm(z[..., Fh:], axis=-1)
        g = jnp.einsum('ts,bsf->btf', w_sp, z2) + b_sp[None, :, None]
        return jnp.einsum('bsf,fd->bsd', z1 * g, w_out)
    x = A_x
    xn = _layernorm(x, axis=-1)
    s = _A_ref(xn, A_w_r, A_w_i)
    g = _silu(_B_ref(xn, B_w_in, B_w_sp, B_b_sp, B_w_out))
    return x + s * g
```

```python
import functools
import math

import numpy as np
import jax
import jax.numpy as jnp
import jax.experimental.pallas as pl
import jax.experimental.pallas.tpu as pltpu

S, D, DF = 2048, 512, 257
FH = 688
EPS = 1e-5
F32, BF16, U32 = jnp.float32, jnp.bfloat16, jnp.uint32
NT = (((1,), (1,)), ((), ()))
RH = math.sqrt(0.5)


@functools.lru_cache(maxsize=None)
def _constants():
    j = np.arange(128)
    lA = 2 * j.copy()
    lA[0] = 256
    lB = 2 * j + 1
    even = (j % 2) == 0
    jn = (j + 1) % 128
    d1 = np.arange(128)[:, None]
    th = lambda l: 2 * np.pi * d1 * l[None, :] / D
    cA, sA = np.cos(th(lA)), np.sin(th(lA))
    sA[:, 0] = 0.0
    G0 = np.where(even[None, :], cA, -sA[:, jn])
    G2 = np.where(~even[None, :], cA, -sA[:, jn])
    sc = 1.0 / (S * D)
    cAT, sAT = cA.T, sA.T
    H0 = np.where(even[:, None], 2 * cAT, -2 * sAT[jn])
    H0[0] = cAT[0]
    H0[127] = 1.0
    H2 = np.where(~even[:, None], 2 * cAT, -2 * sAT[jn])
    mp = (j % 4 == 0) | (j % 4 == 3)
    e = np.arange(64)
    Gp, Gm, Hp, Hm = [np.zeros((128, 128)) for _ in range(4)]
    for jj in range(128):
        l = lB[jj]
        sg = 1.0 if l % 4 == 1 else -1.0
        ang = 2 * np.pi * e * (l if l % 4 == 1 else D - l) / D
        cs, sn = np.cos(ang), np.sin(ang)
        G, H, hi = (Gp, Hp, -1.0) if mp[jj] else (Gm, Hm, 1.0)
        ji = (jj - 2) % 128
        G[:64, jj], G[64:, jj] = cs, hi * sn
        G[:64, ji], G[64:, ji] = -sg * sn, hi * sg * cs
        H[jj, :64], H[jj, 64:] = 2 * cs, 2 * sn
        H[ji, :64], H[ji, 64:] = -2 * sg * sn, 2 * sg * cs
    gf = np.concatenate([G0, G2, Gp, Gm], 1)
    gi = np.concatenate([np.concatenate([H0, H2], 1), np.concatenate([Hp, Hm], 1)], 0) * sc

    k2 = np.arange(16)
    s1 = np.arange(128)
    lam = np.arange(128)
    k1 = 8 * (lam % 16) + lam // 16
    C16 = np.cos(2 * np.pi * np.outer(k2, k2) / 16)
    S16 = np.sin(2 * np.pi * np.outer(k2, k2) / 16)
    Cf = np.cos(2 * np.pi * np.outer(s1, k1) / 128)
    Sf = np.sin(2 * np.pi * np.outer(s1, k1) / 128)
    cm = np.zeros((320, 256))
    cm[0:128] = np.concatenate([Cf, Sf], 1)
    cm[128:256] = np.concatenate([Cf.T, Sf.T], 1)
    cm[256:288, 0:16] = np.concatenate([C16, -S16], 0)
    cm[288:304, 0:32] = np.concatenate([C16, -S16], 1)
    mats = np.concatenate([gi, cm], 0)

    kg = np.arange(256)
    tw = np.zeros((7, 2, 256, 128), np.float32)
    for c in range(1, 8):
        ang = 2 * np.pi * c * kg / S
        tw[c - 1, 0] = np.cos(ang)[:, None]
        tw[c - 1, 1] = np.sin(ang)[:, None]
    angc = 2 * np.pi * np.outer(k2, s1) / S
    small = np.zeros((40, 128), np.float32)
    small[0:16] = np.cos(angc)
    small[16:32] = np.sin(angc)
    return (gf.astype(BF16), mats.astype(BF16), tw.reshape(14, 256, 128), small)


def _sadd(x, y):
    (a, sa), (b, sb) = x, y
    if sa == sb:
        return (a + b, sa)
    return (a - b, 1) if sa > 0 else (b - a, 1)


def _sneg(x):
    return (x[0], -x[1])


def _ssub(x, y):
    return _sadd(x, _sneg(y))


def _smul(x, c):
    return (x[0] * (float(c) * x[1]), 1)


def _val(x):
    return x[0] if x[1] > 0 else -x[0]


def _cadd(u, v):
    return (_sadd(u[0], v[0]), _sadd(u[1], v[1]))


def _csub(u, v):
    return (_ssub(u[0], v[0]), _ssub(u[1], v[1]))


def _crot(u, num, den):
    num = num % den
    re, im = u
    if num == 0:
        return u
    if 2 * num == den:
        return (_sneg(re), _sneg(im))
    if 4 * num == den:
        return (im, _sneg(re))
    if 4 * num == 3 * den:
        return (_sneg(im), re)
    if (8 * num) % den == 0:
        q = (8 * num) // den
        r = math.sqrt(0.5)
        c, s = (r, r) if q == 1 else (-r, r) if q == 3 else (-r, -r) if q == 5 else (r, -r)
        if c * s > 0:
            return (_smul(_sadd(re, im), c), _smul(_ssub(im, re), c))
        return (_smul(_ssub(re, im), c), _smul(_sadd(im, re), c))
    c, s = math.cos(2 * math.pi * num / den), math.sin(2 * math.pi * num / den)
    return (_sadd(_smul(re, c), _smul(im, s)), _ssub(_smul(im, c), _smul(re, s)))


def _dft(vs, sign):
    n = len(vs)
    if n == 1:
        return vs
    h = n // 2
    a = [_cadd(vs[i], vs[i + h]) for i in range(h)]
    b = [_crot(_csub(vs[i], vs[i + h]), sign * i, n) for i in range(h)]
    ea, eb = _dft(a, sign), _dft(b, sign)
    out = [None] * n
    out[0::2] = ea
    out[1::2] = eb
    return out


def _cx(re, im):
    return ((re, 1), (im, 1))


def _cmul_vec(u, c, s, conj):
    (re, sr), (im, si) = u
    rc, is_, ic, rs = (re * c, sr), (im * s, si), (im * c, si), (re * s, sr)
    if not conj:
        return (_sadd(rc, is_), _ssub(ic, rs))
    return (_ssub(rc, is_), _sadd(ic, rs))


def _gelu2(x):
    c = math.sqrt(2.0 / math.pi)
    return x + x * jnp.tanh(x * (c + (c * 0.044715) * (x * x)))


def _pack(x):
    return pltpu.bitcast(x.astype(BF16), U32)


def _unpack(x):
    return pltpu.bitcast(x, BF16)


def _kernel(x_hbm, wr_hbm, wi_hbm, win_hbm, wsp_hbm, b_hbm, wout_hbm,
            gf_hbm, mats_hbm, tw_hbm, small_hbm, out_hbm,
            x_s, xn_f, win_f, z1_f, z2n_f, wsp_s, b1_f, b2_f, b3_f, b4_f, wraw_s, wt_f,
            gf_s, mats_s, tw_f, small_s, b_s, wout_s, woT_f, a2_s, st_f, o_f, out_s,
            sems, zsem):
    x32 = x_hbm.bitcast(U32)
    cnt = [0]
    z0 = pl.semaphore_read(zsem)

    def dyn(ref):
        cnt[0] += 1
        return ref.at[z0 * (cnt[0] + 1)]

    xn_s, z1_s, z2n_s, b1_s, wt_s = xn_f.at[z0], z1_f.at[z0], z2n_f.at[z0], b1_f.at[z0], wt_f.at[z0]
    st_s, o_s, woT_s, b2_s = st_f.at[z0], o_f.at[z0], woT_f.at[z0], b2_f.at[z0]
    b3_s, b4_s = b3_f.at[z0], b4_f.at[z0]
    win_s, tw_s = win_f.at[0], tw_f.at[0]

    def cp(src, dst, i):
        return pltpu.make_async_copy(src, dst, sems.at[i])

    x_cps = [[cp(x32.at[pl.ds(2 * hf, 2), pl.ds(0, 64), :], x_s.at[pl.ds(2 * hf, 2), pl.ds(0, 64), :], 4 + hf)
              for hf in range(2)]]
    x_cps += [[cp(x32.at[:, pl.ds(64 * i, 64), :], x_s.at[:, pl.ds(64 * i, 64), :], i)] for i in range(1, 4)]
    c_gf = cp(gf_hbm.bitcast(U32), gf_s, 16)
    c_small = cp(small_hbm, small_s, 17)
    win32 = win_hbm.bitcast(U32)
    c_win2 = cp(win32.at[pl.ds(FH // 2, FH // 2), :], win_s.at[pl.ds(FH // 2, FH // 2), :], 18)
    c_win1 = cp(win32.at[pl.ds(0, FH // 2), :], win_s.at[pl.ds(0, FH // 2), :], 43)
    wsp32 = wsp_hbm.bitcast(U32)
    wsp_edges = [0, 2, 4, 8, 9, 11, 12, 16]
    c_wsp = [cp(wsp32.at[pl.ds(64 * lo, 64 * (hi - lo)), :], wsp_s.at[pl.ds(64 * lo, 64 * (hi - lo)), :], 44 + q)
             for q, (lo, hi) in enumerate(zip(wsp_edges[:-1], wsp_edges[1:]))]
    c_wr = cp(wr_hbm, wraw_s.at[0], 21)
    c_wi = cp(wi_hbm, wraw_s.at[1], 22)
    c_tw = cp(tw_hbm, tw_s, 23)
    c_mats = cp(mats_hbm.bitcast(U32), mats_s, 24)
    c_b = cp(b_hbm, b_s, 25)
    c_wout = cp(wout_hbm, wout_s, 26)
    out_cps = [cp(out_s.at[pl.ds(128 * t, 128), :], out_hbm.at[0, pl.ds(128 * t, 128), :], 27 + t)
               for t in range(16)]

    for c in [x_cps[0][0], c_win2, x_cps[0][1], c_win1] + x_cps[1] + [c_gf] + x_cps[2] + x_cps[3] + [
            c_wr, c_wi, c_wout, c_b, c_small, c_wsp[0], c_mats, c_wsp[1], c_tw] + c_wsp[2:]:
        c.start()

    lane = jax.lax.broadcasted_iota(jnp.int32, (8, 128), 1)

    def lane_mask(n, kind="even"):
        ln = jax.lax.broadcasted_iota(jnp.int32, (n, 128), 1)
        if kind == "even":
            return (ln & 1) == 0
        if kind == "lo":
            return ln < 64
        return ((ln + 1) & 2) == 0

    row16 = jax.lax.broadcasted_iota(jnp.int32, (16, 512), 0)
    win_s[pl.ds(FH, 8), :] = _pack(jnp.where(row16 == 0, 1.0, 0.0).astype(F32))

    zero = jnp.full((8, 128), z0, jnp.int32).astype(U32)

    def mask0(dep):
        reps = dep.shape[-2] // 8
        z = zero if reps == 1 else jnp.concatenate([zero] * reps, axis=0)
        z = jnp.broadcast_to(z, dep.shape) if dep.ndim > 2 else z
        return pltpu.bitcast(dep, U32) & z

    def tie0(v, d):
        if v.dtype == U32:
            return v | d
        return pltpu.bitcast(pltpu.bitcast(v, U32) | d, F32)

    def tie(v, dep):
        return tie0(v, mask0(dep))

    def ctie(u, d, both=True):
        (re, sr), (im, si) = u
        return ((tie0(re, d), sr), (tie0(im, d) if both else im, si))

    def pick(rs, n):
        tot = sum(r.shape[0] // 8 for r in rs)
        out = []
        for u in range(n):
            g = (u * tot) // n
            for r in rs:
                m = r.shape[0] // 8
                if g < m:
                    out.append(r[8 * g:8 * g + 8, 0:128])
                    break
                g -= m
        return out

    US = {}

    def pre(i, e, xb):
        xf = xb.astype(F32)
        x0, x1, x2, x3 = [xf[:, 128 * k:128 * (k + 1)] for k in range(4)]
        s02, s13 = x0 + x2, x1 + x3
        p, q = x0 - x2, x1 - x3
        lo = lane_mask(128, "lo")
        sv = jnp.where(lo, p, (p + q) * RH)
        rc = pltpu.roll(jnp.where(lo, q, (p - q) * RH), 64, 1)
        US[i, e] = tuple(t.astype(BF16) for t in (s02 + s13, s02 - s13, sv + rc, sv - rc))

    def ln1(i, es, deps=None):
        for n, e in enumerate(es):
            x = _unpack(x_s[e, pl.ds(64 * i, 64), :]).astype(F32)
            m = jnp.sum(x, axis=1, keepdims=True) * (1.0 / D)
            xc = x - m
            v = jnp.sum(xc * xc, axis=1, keepdims=True) * (1.0 / D)
            rstd = jnp.broadcast_to(jax.lax.rsqrt(v + EPS), (128, 128))
            if deps is not None:
                rstd = tie(rstd, jnp.concatenate(deps[16 * n:16 * n + 16], axis=0))
            xb = (xc * jnp.concatenate([rstd] * 4, axis=1)).astype(BF16)
            xn_s[pl.ds(256 * e + 64 * i, 64), :] = pltpu.bitcast(xb, U32)
            pre(i, e, xb)

    def dfwd(i):
        us = [jnp.concatenate([US[i, e][k][16 * r:16 * r + 16] for r in range(8) for e in range(4)], axis=0)
              for k in range(4)]
        gf = _unpack(gf_s[...])
        o0, o2, op, om = [jnp.dot(us[k], gf[:, 128 * k:128 * (k + 1)], preferred_element_type=F32)
                          for k in range(4)]
        ev, mp = lane_mask(512), lane_mask(512, "mp")
        re = jnp.stack([jnp.where(ev, o0, o2), jnp.where(mp, op, om)])
        im = jnp.stack([pltpu.roll(jnp.where(ev, o2, o0), 1, 1), pltpu.roll(jnp.where(mp, om, op), 2, 1)])
        re = re.reshape(2, 8, 4, 2, 8, 128)
        im = im.reshape(2, 8, 4, 2, 8, 128)
        outs = _dft([_cx(re[:, :, e], im[:, :, e]) for e in range(4)], 1)
        for ke in range(4):
            for ri in range(2):
                b1_s[ri, :, pl.ds(2 * i, 2), ke] = _val(outs[ke][ri]).reshape(2, 2, 8, 8, 128)

    def zt2(sig):
        lhs = _unpack(dyn(win_f)[pl.ds(FH // 2, FH // 2 + 8), :])
        rhs = _unpack(xn_s[pl.ds(64 * sig, 64), :])
        r = jax.lax.dot_general(lhs, rhs, NT, preferred_element_type=F32)
        z2 = _gelu2(r[0:FH])
        a2_s[pl.ds(sig, 1), :] = r[FH:FH + 1]
        mu = jnp.sum(z2, axis=0, keepdims=True) * (1.0 / FH)
        ms = jnp.sum(z2 * z2, axis=0, keepdims=True) * (1.0 / FH)
        var = jnp.maximum(ms - mu * mu, 0.0)
        rstd = jnp.broadcast_to(jax.lax.rsqrt(var + 4.0 * EPS), (8, 128))
        mr = jnp.broadcast_to(mu, (8, 128)) * rstd

        def norm(deps=None):
            edges = [0, 96, 176, 272, 352, 448, 528, 624, FH]
            for q in range(8):
                n = (edges[q + 1] - edges[q]) // 8
                rq = rstd if deps is None else tie(rstd, deps[q])
                zq = z2[edges[q]:edges[q + 1]] * jnp.concatenate([rq] * n, axis=0) - jnp.concatenate([mr] * n, axis=0)
                z2n_s[pl.ds(edges[q] // 2, 4 * n), pl.ds(128 * sig, 128)] = _pack(zq)
        return r, norm

    def zt1(sig):
        lhs = _unpack(dyn(win_f)[pl.ds(0, FH // 2), :])
        rhs = _unpack(xn_s[pl.ds(64 * sig, 64), :])
        r = jax.lax.dot_general(lhs, rhs, NT, preferred_element_type=F32)
        z1_s[sig] = _gelu2(r)
        return r

    pend = []

    def run(piece, sig):
        out = piece(sig)
        r = out[0] if piece is zt2 else out
        while pend:
            pend.pop()(pick([r], 8))
        if piece is zt2:
            pend.append(out[1])
        return r

    def flush():
        while pend:
            pend.pop()()

    x_cps[0][0].wait()
    ln1(0, (0, 1))
    c_win2.wait()
    x_cps[0][1].wait()
    ln1(0, (2, 3), pick([run(zt2, 0), run(zt2, 4)[0:352]], 32))
    run(zt2, 8)
    run(zt2, 12)
    c_win1.wait()
    x_cps[1][0].wait()
    rs = [run(zt1, 4 * e) for e in range(4)]
    ln1(1, (0, 1), pick(rs[:3], 32))
    c_gf.wait()
    for i in (2, 3):
        for c in x_cps[i]:
            c.wait()
    dfwd(0)
    rs = [run(zt, sig) for sig in (1, 5) for zt in (zt2, zt1)]
    ln1(1, (2, 3), pick(rs[:3], 32))
    rs = [run(zt, sig) for sig in (9, 13) for zt in (zt2, zt1)]
    ln1(2, (0, 1, 2, 3), pick(rs, 64))
    dfwd(1)
    rs = [run(zt, sig) for sig in (2, 6, 10) for zt in (zt2, zt1)]
    ln1(3, (0, 1, 2, 3), pick(rs[:5], 64))
    dfwd(2)
    run(zt2, 14)
    dfwd(3)
    run(zt1, 14)

    for c in (c_wr, c_wi, c_wout, c_b, c_small, c_wsp[0], c_mats):
        c.wait()

    links = []

    def wprep(deps):
        row = jax.lax.broadcasted_iota(jnp.int32, (16, 128), 0)
        for p in range(2):
            for kb in range(16):
                cols = pl.ds(128 * kb, 128)
                top = wraw_s[p, pl.ds(0, 16), cols].astype(F32)
                ny = wraw_s[p, pl.ds(256, 1), cols].astype(F32)
                top = jnp.where(row == 0, jnp.broadcast_to(ny, (16, 128)), top)
                d = deps[16 * p + kb]
                blk = jnp.concatenate([tie(_pack(top), d),
                                       pltpu.bitcast(wraw_s[p, pl.ds(16, 240), cols], U32)], axis=0)
                bt = blk.T
                wt_s[p, pl.ds(128 * kb, 128), :] = bt
                links.append(bt[120:128])

    def woprep(deps):
        w = pltpu.bitcast(wout_s[...], U32)
        cols = []
        for cb in range(4):
            rows = []
            for rb in range(6):
                blk = w[64 * rb:min(64 * rb + 64, FH // 2), 128 * cb:128 * cb + 128]
                rows += [tie(blk[0:8], deps[6 * cb + rb]), blk[8:]]
            cols.append(jnp.concatenate(rows, axis=0))
        woT_s[...] = pltpu.bitcast(_unpack(jnp.concatenate(cols, axis=1)).T, U32)

    def compact():
        mats = _unpack(mats_s[pl.ds(128, 160), :])
        mf, mi = mats[0:128], mats[128:256]
        f16, i16 = mats[256:288, 0:16], mats[288:304, 0:32]
        tc, ts = small_s[pl.ds(0, 16), :], small_s[pl.ds(16, 16), :]
        u = jnp.dot(f16, a2_s[...].astype(BF16), preferred_element_type=F32)
        ur, ui = u[0:16], u[16:32]
        ur, ui = ur * tc + ui * ts, ui * tc - ur * ts
        yield None
        r = jnp.dot(jnp.concatenate([ur, ui], axis=0).astype(BF16), mf, preferred_element_type=F32)
        pr, pi = r[0:16, 0:128] + r[16:32, 128:256], r[16:32, 0:128] - r[0:16, 128:256]
        blk = jax.lax.broadcasted_iota(jnp.int32, (16, 128), 1) // 16
        w0 = []
        for p in range(2):
            wn = jnp.concatenate([wraw_s[p, pl.ds(0, 8), pl.ds(128 * be, 128)].astype(F32)[0:1]
                                  for be in range(16)], axis=0)
            tf = jnp.concatenate([wn] * 8, axis=0).T
            acc = tf[0:16]
            for ka in range(1, 8):
                acc = jnp.where(blk == ka, tf[16 * ka:16 * ka + 16], acc)
            w0.append(acc)
        yr, yi = pr * w0[0] - pi * w0[1], pr * w0[1] + pi * w0[0]
        yield None
        r = jnp.dot(jnp.concatenate([yr, yi], axis=0).astype(BF16), mi, preferred_element_type=F32)
        vr, vi = r[0:16, 0:128] - r[16:32, 128:256], r[16:32, 0:128] + r[0:16, 128:256]
        vr, vi = vr * tc - vi * ts, vi * tc + vr * ts
        yield None
        ap = jnp.dot(i16, jnp.concatenate([vr, vi], axis=0).astype(BF16), preferred_element_type=F32)
        yield jnp.concatenate([ap] * 8, axis=0).T

    def split(deps, shape):
        return [mask0(jnp.concatenate(deps[k::2], axis=0).reshape(shape)) for k in range(2)]

    def tied(ins, d):
        ins[1], ins[0] = ctie(ins[1], d[0]), ctie(ins[0], d[1])
        return ins

    def p2(deps):
        for ke in range(4):
            for b in range(8):
                n = 4 * (8 * ke + b)
                ins = tied([_cx(b1_s[0, :, a, ke, b], b1_s[1, :, a, ke, b]) for a in range(8)],
                           split(deps[n:n + 4], (2, 8, 128)))
                outs = _dft([_crot(ins[a], (8 * a + b) * ke, 256) for a in range(8)], 1)
                for ka in range(8):
                    for ri in range(2):
                        b3_s[ri, :, ka, ke, b] = _val(outs[ka][ri])

    def p3(deps):
        for ka in range(8):
            ins = tied([_cx(b3_s[0, :, ka, :, b], b3_s[1, :, ka, :, b]) for b in range(8)],
                       split(deps[16 * ka:16 * ka + 16], (2, 4, 8, 128)))
            outs = _dft([_crot(ins[b], b * ka, 64) for b in range(8)], 1)
            for kb in range(8):
                for ri in range(2):
                    b2_s[ri, :, pl.ds(256 * kb + 32 * ka, 32), :] = _val(outs[kb][ri]).reshape(2, 32, 128)

    def mid(t, deps):
        d = [mask0(jnp.concatenate(deps[k::5], axis=0)) for k in range(5)]
        twa, twb, wt = dyn(tw_f), dyn(tw_f), dyn(wt_f)
        ins = []
        for c in range(8):
            u = _cx(b2_s[0, t, pl.ds(c, 256, stride=8), :], b2_s[1, t, pl.ds(c, 256, stride=8), :])
            if c < 2:
                u = ctie(u, d[1 - c], both=(c == 0))
            ins.append(u if c == 0 else _cmul_vec(u, twa[2 * c - 2], twa[2 * c - 1], False))
        outs = _dft(ins, 1)
        sel = [d[3 - k] | jnp.uint32(16 if t == 0 else 0xFFFF0000) for k in range(2)]
        ys = []
        for kc in range(8):
            wr, wi = wt[0, pl.ds(256 * kc, 256), :], wt[1, pl.ds(256 * kc, 256), :]
            if t == 0:
                wr, wi = wr << sel[kc % 2], wi << sel[kc % 2]
            else:
                wr, wi = wr & sel[kc % 2], wi & sel[kc % 2]
            ys.append(_cmul_vec(outs[kc], pltpu.bitcast(wr, F32), pltpu.bitcast(wi, F32), True))
        outs = _dft(ys, -1)
        for c in range(8):
            o = outs[c] if c == 0 else _cmul_vec(outs[c], tie0(twb[2 * c - 2], d[4]), twb[2 * c - 1], True)
            b4_s[0, t, pl.ds(c, 256, stride=8), :] = _val(o[0])
            b4_s[1, t, pl.ds(c, 256, stride=8), :] = _val(o[1])

    def p3i(deps):
        ins = tied([_cx(b4_s[0, :, pl.ds(256 * kb, 256), :], b4_s[1, :, pl.ds(256 * kb, 256), :])
                    for kb in range(8)], split(deps, (2, 256, 128)))
        outs = _dft(ins, -1)
        for b in range(8):
            for ri in range(2):
                b1_s[ri, :, :, :, b] = _val(outs[b][ri]).reshape(2, 8, 4, 8, 128)

    def p2i(deps):
        for b in range(8):
            ins = tied([_cx(b1_s[0, :, ka, :, b], b1_s[1, :, ka, :, b]) for ka in range(8)],
                       split(deps[16 * b:16 * b + 16], (2, 4, 8, 128)))
            outs = _dft([_crot(ins[ka], -b * ka, 64) for ka in range(8)], -1)
            for a in range(8):
                for ri in range(2):
                    b3_s[ri, :, a, :, b] = _val(outs[a][ri])

    def p1i(deps, apT):
        ev, mp = lane_mask(16), lane_mask(16, "mp")
        l0 = jax.lax.broadcasted_iota(jnp.int32, (16, 128), 1) == 0
        for a in range(8):
            for bp in range(4):
                n = 4 * a + bp
                d = split(deps[4 * n:4 * n + 4], (2, 8, 128))
                res = []
                for hh in range(2):
                    b = 2 * bp + hh
                    ins = [_cx(b3_s[0, :, a, ke, b], b3_s[1, :, a, ke, b]) for ke in range(4)]
                    ins[0] = ctie(ins[0], d[hh])
                    res.append(_dft([_crot(ins[ke], -(8 * a + b) * ke, 256) for ke in range(4)], -1))
                r0 = 64 * a + 16 * bp
                for e in range(4):
                    re = jnp.concatenate([_val(res[0][e][0]), _val(res[1][e][0])], axis=1)
                    im = jnp.concatenate([_val(res[0][e][1]), _val(res[1][e][1])], axis=1)
                    s2 = 4 * e + r0 // 128
                    col = jnp.broadcast_to(apT[r0 % 128:r0 % 128 + 16, s2:s2 + 1], (16, 128))
                    ri = pltpu.roll(jnp.where(l0, col, im[0]), 127, 1)
                    i0, i2 = jnp.where(ev, re[0], ri), jnp.where(ev, ri, re[0])
                    rb = pltpu.roll(im[1], 126, 1)
                    ip, in_ = jnp.where(mp, re[1], rb), jnp.where(mp, rb, re[1])
                    st_s[pl.ds(256 * e + r0 // 2, 8), :] = _pack(jnp.concatenate([i0, i2, ip, in_], axis=1))

    def gt_pieces(t, hook=None):
        rs = []
        z2n = dyn(z2n_f)
        held = list(links)
        del links[:]
        for kg in range(4):
            rs.append(jax.lax.dot_general(_unpack(z2n[:, pl.ds(512 * kg, 512)]),
                                          _unpack(wsp_s[pl.ds(64 * t, 64), pl.ds(512 * kg, 512)]),
                                          NT, preferred_element_type=F32))
            if hook is not None:
                hook(kg)
        r0 = rs[0]
        if held:
            acc = held.pop()
            while held:
                acc = acc | held.pop()
            r0 = jnp.concatenate([r0[0:480], tie0(r0[480:488], acc & zero), r0[488:]], axis=0)
        g = r0 + rs[1] + rs[2] + rs[3] + b_s[pl.ds(t, 1), :].astype(F32)
        h = (z1_s[t] * g).astype(BF16)
        return rs, h

    def bout(t, h):
        wo = dyn(woT_f)
        oT = jnp.concatenate([jnp.dot(_unpack(wo[pl.ds(128 * q, 128), :]), h, preferred_element_type=F32)
                              for q in range(2)], axis=0)
        ho = 0.25 * oT
        gate = ho + ho * jnp.tanh(ho)
        gT = pltpu.bitcast(gate.astype(BF16).T, U32)
        o_s[pl.ds(64 * t, 64), :] = gT
        links.extend([gT[56:64, 128 * q:128 * q + 128] for q in range(4)])
        return oT

    def final(t):
        gi = _unpack(mats_s[pl.ds(0, 128), :])
        z = _unpack(st_s[pl.ds(64 * t, 64), :])
        v0, v2, tp, tm = [jnp.dot(z[:, 128 * k:128 * (k + 1)],
                                  gi[128 * (k // 2):128 * (k // 2) + 128, 128 * (k % 2):128 * (k % 2) + 128],
                                  preferred_element_type=F32) for k in range(4)]
        sp, sm = v0 + v2, v0 - v2
        ss, df = tp + tm, tp - tm
        lo = lane_mask(128, "lo")
        rc = pltpu.roll(jnp.where(lo, df, ss), 64, 1)
        pp, qn = jnp.where(lo, ss, (rc - df) * RH), jnp.where(lo, rc, (rc + df) * RH)
        y = jnp.concatenate([sp + pp, sm - qn, sp - pp, sm + qn], axis=1)
        gate = _unpack(o_s[pl.ds(64 * t, 64), :]).astype(F32)
        x = _unpack(x_s[t // 4, pl.ds(64 * (t % 4), 64), :]).astype(F32)
        out_s[pl.ds(128 * t, 128), :] = (x + y * gate).astype(BF16)
        out_cps[t].start()

    ra = [run(zt2, 3), run(zt2, 7), run(zt2, 11), run(zt2, 15)]
    rb = [run(zt1, 3), run(zt1, 7), run(zt1, 11), run(zt1, 15)]
    woprep(pick(ra, 24))
    wprep(pick(ra + rb, 32))

    R, H = {}, {}
    cgen = compact()
    cres = []

    def gt(t, hook=None):
        R[t], H[t] = gt_pieces(t, hook)

    def early(rs):
        return rs[:-1] + [rs[-1][0:432]]

    gt(0)
    bout(0, H[0])
    gt(1)
    p2(pick(early(R[0] + R[1]), 128))

    c_wsp[1].wait()
    next(cgen)
    gt(2)
    bout(1, H[1])
    bout(2, H[2])
    gt(3)
    p3(pick(early(R[2] + R[3]), 128))

    c_wsp[2].wait()
    c_tw.wait()
    next(cgen)
    gt(4)
    bout(3, H[3])
    gt(5)
    bout(4, H[4])
    mid(0, pick(R[4] + R[5], 160))
    gt(6)
    bout(5, H[5])
    bout(6, H[6])
    gt(7)
    mid(1, pick(early(R[6] + R[7]), 160))

    c_wsp[3].wait()
    next(cgen)
    gt(8)
    p3i(pick(early(R[8]), 128))

    c_wsp[4].wait()
    apT = next(cgen)
    gt(9)
    bout(7, H[7])
    bout(8, H[8])
    bout(9, H[9])
    gt(10)
    p2i(pick(early(R[9] + R[10]), 128))

    c_wsp[5].wait()
    gt(11)
    p1i(pick(early(R[11]), 128), apT)

    c_wsp[6].wait()
    gt(12)
    bout(10, H[10])
    bout(11, H[11])
    for t in (13, 14, 15):
        gt(t, lambda kg: final(4 * (t - 13) + kg))
        bout(t - 1, H[t - 1])
    final(12)
    final(13)
    bout(15, H[15])
    final(14)
    final(15)
    for c in out_cps:
        c.wait()


@jax.jit
def pallas_recurrent_scan__spectral_gfnet__mixer_gmlp__prompt_kernel(
    A_x: jax.Array,
    A_w_r: jax.Array,
    A_w_i: jax.Array,
    B_x: jax.Array,
    B_w_in: jax.Array,
    B_w_sp: jax.Array,
    B_b_sp: jax.Array,
    B_w_out: jax.Array,
):
    gf, mats, tw, small = _constants()
    args = (A_x.reshape(4, 512, 512), A_w_r.T, A_w_i.T, B_w_in.T, B_w_sp, B_b_sp.reshape(16, 128), B_w_out,
            jnp.asarray(gf), jnp.asarray(mats), jnp.asarray(tw), jnp.asarray(small))
    vm = pltpu.VMEM
    scratch = [
        vm((4, 256, 512), U32),
        vm((1, 1024, 512), U32),
        vm((1, FH + 8, 512), U32),
        vm((1, 16, FH, 128), F32),
        vm((1, FH // 2, 2048), U32),
        vm((1024, 2048), U32),
        vm((1, 2, 2, 8, 4, 8, 8, 128), F32),
        vm((1, 2, 2, 2048, 128), F32),
        vm((1, 2, 2, 8, 4, 8, 8, 128), F32),
        vm((1, 2, 2, 2048, 128), F32),
        vm((2, DF, 2048), BF16),
        vm((1, 2, 2048, 128), U32),
        vm((64, 512), U32),
        vm((288, 256), U32),
        vm((1, 14, 256, 128), F32),
        vm((40, 128), F32),
        vm((16, 128), BF16),
        vm((FH, 512), BF16),
        vm((1, 256, FH), U32),
        vm((16, 128), F32),
        vm((1, 1024, 512), U32),
        vm((1, 1024, 512), U32),
        vm((2048, 512), BF16),
        pltpu.SemaphoreType.DMA((51,)),
        pltpu.SemaphoreType.REGULAR,
    ]
    return pl.pallas_call(
        _kernel,
        out_shape=jax.ShapeDtypeStruct((1, S, D), BF16),
        in_specs=[pl.BlockSpec(memory_space=pl.ANY)] * len(args),
        out_specs=pl.BlockSpec(memory_space=pl.ANY),
        scratch_shapes=scratch,
        compiler_params=pltpu.CompilerParams(vmem_limit_bytes=100 * 1024 * 1024,
                                             disable_semaphore_checks=True, disable_bounds_checks=True),
    )(*args)
```

```python
import functools
import math

import numpy as np
import jax
import jax.numpy as jnp
import jax.experimental.pallas as pl
import jax.experimental.pallas.tpu as pltpu

S, D, DF = 2048, 512, 257
FH = 688
HM = 352
EPS = 1e-5
F32, BF16, U32 = jnp.float32, jnp.bfloat16, jnp.uint32
NT = (((1,), (1,)), ((), ()))
RH = math.sqrt(0.5)


@functools.lru_cache(maxsize=None)
def _constants():
    j = np.arange(128)
    lA = 2 * j.copy()
    lA[0] = 256
    lB = 2 * j + 1
    even = (j % 2) == 0
    jn = (j + 1) % 128
    d1 = np.arange(128)[:, None]
    th = lambda l: 2 * np.pi * d1 * l[None, :] / D
    cA, sA = np.cos(th(lA)), np.sin(th(lA))
    sA[:, 0] = 0.0
    G0 = np.where(even[None, :], cA, -sA[:, jn])
    G2 = np.where(~even[None, :], cA, -sA[:, jn])
    sc = 1.0 / (S * D)
    cAT, sAT = cA.T, sA.T
    H0 = np.where(even[:, None], 2 * cAT, -2 * sAT[jn])
    H0[0] = cAT[0]
    H0[127] = 1.0
    H2 = np.where(~even[:, None], 2 * cAT, -2 * sAT[jn])
    mp = (j % 4 == 0) | (j % 4 == 3)
    e = np.arange(64)
    Gp, Gm, Hp, Hm = [np.zeros((128, 128)) for _ in range(4)]
    for jj in range(128):
        l = lB[jj]
        sg = 1.0 if l % 4 == 1 else -1.0
        ang = 2 * np.pi * e * (l if l % 4 == 1 else D - l) / D
        cs, sn = np.cos(ang), np.sin(ang)
        G, H, hi = (Gp, Hp, -1.0) if mp[jj] else (Gm, Hm, 1.0)
        ji = (jj - 2) % 128
        G[:64, jj], G[64:, jj] = cs, hi * sn
        G[:64, ji], G[64:, ji] = -sg * sn, hi * sg * cs
        H[jj, :64], H[jj, 64:] = 2 * cs, 2 * sn
        H[ji, :64], H[ji, 64:] = -2 * sg * sn, 2 * sg * cs
    gf = np.concatenate([G0, G2, Gp, Gm], 1)
    gi = np.concatenate([np.concatenate([H0, H2], 1), np.concatenate([Hp, Hm], 1)], 0) * sc

    k2 = np.arange(16)
    s1 = np.arange(128)
    lam = np.arange(128)
    k1 = 8 * (lam % 16) + lam // 16
    C16 = np.cos(2 * np.pi * np.outer(k2, k2) / 16)
    S16 = np.sin(2 * np.pi * np.outer(k2, k2) / 16)
    Cf = np.cos(2 * np.pi * np.outer(s1, k1) / 128)
    Sf = np.sin(2 * np.pi * np.outer(s1, k1) / 128)
    cm = np.zeros((320, 256))
    cm[0:128] = np.concatenate([Cf, Sf], 1)
    cm[128:256] = np.concatenate([Cf.T, Sf.T], 1)
    cm[256:288, 0:16] = np.concatenate([C16, -S16], 0)
    cm[288:304, 0:32] = np.concatenate([C16, -S16], 1)
    mats = np.concatenate([gi, cm], 0)

    kg = np.arange(256)
    tw = np.zeros((7, 2, 256, 128), np.float32)
    for c in range(1, 8):
        ang = 2 * np.pi * c * kg / S
        tw[c - 1, 0] = np.cos(ang)[:, None]
        tw[c - 1, 1] = np.sin(ang)[:, None]
    angc = 2 * np.pi * np.outer(k2, s1) / S
    small = np.zeros((40, 128), np.float32)
    small[0:16] = np.cos(angc)
    small[16:32] = np.sin(angc)

    def packed(m):
        b = np.asarray(m.astype(BF16)).view(np.uint16).astype(np.uint32)
        return b[0::2] | (b[1::2] << 16)
    return (packed(gf), packed(mats), tw.reshape(14, 256, 128), small)


def _sadd(x, y):
    (a, sa), (b, sb) = x, y
    if sa == sb:
        return (a + b, sa)
    return (a - b, 1) if sa > 0 else (b - a, 1)


def _sneg(x):
    return (x[0], -x[1])


def _ssub(x, y):
    return _sadd(x, _sneg(y))


def _smul(x, c):
    return (x[0] * (float(c) * x[1]), 1)


def _val(x):
    return x[0] if x[1] > 0 else -x[0]


def _cadd(u, v):
    return (_sadd(u[0], v[0]), _sadd(u[1], v[1]))


def _csub(u, v):
    return (_ssub(u[0], v[0]), _ssub(u[1], v[1]))


def _crot(u, num, den):
    num = num % den
    re, im = u
    if num == 0:
        return u
    if 2 * num == den:
        return (_sneg(re), _sneg(im))
    if 4 * num == den:
        return (im, _sneg(re))
    if 4 * num == 3 * den:
        return (_sneg(im), re)
    if (8 * num) % den == 0:
        q = (8 * num) // den
        r = math.sqrt(0.5)
        c, s = (r, r) if q == 1 else (-r, r) if q == 3 else (-r, -r) if q == 5 else (r, -r)
        if c * s > 0:
            return (_smul(_sadd(re, im), c), _smul(_ssub(im, re), c))
        return (_smul(_ssub(re, im), c), _smul(_sadd(im, re), c))
    c, s = math.cos(2 * math.pi * num / den), math.sin(2 * math.pi * num / den)
    return (_sadd(_smul(re, c), _smul(im, s)), _ssub(_smul(im, c), _smul(re, s)))


def _dft(vs, sign):
    n = len(vs)
    if n == 1:
        return vs
    h = n // 2
    a = [_cadd(vs[i], vs[i + h]) for i in range(h)]
    b = [_crot(_csub(vs[i], vs[i + h]), sign * i, n) for i in range(h)]
    ea, eb = _dft(a, sign), _dft(b, sign)
    out = [None] * n
    out[0::2] = ea
    out[1::2] = eb
    return out


def _cx(re, im):
    return ((re, 1), (im, 1))


def _cmul_vec(u, c, s, conj):
    (re, sr), (im, si) = u
    rc, is_, ic, rs = (re * c, sr), (im * s, si), (im * c, si), (re * s, sr)
    if not conj:
        return (_sadd(rc, is_), _ssub(ic, rs))
    return (_ssub(rc, is_), _sadd(ic, rs))


def _gelu2(x):
    c = math.sqrt(2.0 / math.pi)
    return x + x * jnp.tanh(x * (c + (c * 0.044715) * (x * x)))


def _rsqrt(v):
    y = pltpu.bitcast(jnp.uint32(0x5F3759DF) - (pltpu.bitcast(v, U32) >> 1), F32)
    hv = 0.5 * v
    for _ in range(3):
        y = y * (1.5 - hv * (y * y))
    return y


def _pack(x):
    return pltpu.bitcast(x.astype(BF16), U32)


def _unpack(x):
    return pltpu.bitcast(x, BF16)


def _up(x):
    return _unpack(x).astype(F32)


def _kernel(x_hbm, wr_hbm, wi_hbm, win_hbm, wsp_hbm, b_hbm, wout_hbm,
            gf_hbm, mats_hbm, tw_hbm, small_hbm, zero_hbm, out_hbm,
            x_s, xn_f, win_f, wsum_f, xs_f, z1_f, aop_f, wsp_f, b1_f, b2_f, b4_f, wraw_s, wt_f,
            gf_s, mats_s, tw_f, small_s, b_s, wout_s, woT_f, a2_s, ac_f, st_f, o_f, out_s,
            zero_s, sems):
    cnt = [0]
    win_s, tw_s, wsp_s = win_f.at[0], tw_f.at[0], wsp_f.at[0]

    def cp(src, dst, i):
        return pltpu.make_async_copy(src, dst, sems.at[i])

    x_cps = [[cp(x_hbm.at[pl.ds(lo, 2), pl.ds(0, 128), :], x_s.at[pl.ds(lo, 2), pl.ds(0, 128), :], 4 + lo)
              for lo in (0, 2)]]
    x_cps += [[cp(x_hbm.at[e, pl.ds(128, 128), :], x_s.at[e, pl.ds(128, 128), :], 11 + e) for e in (0, 2, 1, 3)]]
    x_cps += [[cp(x_hbm.at[:, pl.ds(128 * i, 128), :], x_s.at[:, pl.ds(128 * i, 128), :], i)] for i in range(2, 4)]
    c_gf = cp(gf_hbm, gf_s, 16)
    c_small = cp(small_hbm, small_s, 17)
    c_win2 = cp(win_hbm.at[pl.ds(FH, HM), :], win_s.at[pl.ds(2 * HM, HM), :], 18)
    c_win2b = cp(win_hbm.at[pl.ds(FH + HM, FH - HM), :], win_s.at[pl.ds(3 * HM, FH - HM), :], 20)
    c_win1 = cp(win_hbm.at[pl.ds(0, FH), :], win_s.at[pl.ds(0, FH), :], 43)
    wsp_edges = [0, 3, 5, 8]
    c_wsp = [cp(wsp_hbm.at[:, pl.ds(128 * lo, 128 * (hi - lo)), :], wsp_s.at[:, pl.ds(128 * lo, 128 * (hi - lo)), :], 44 + q)
             for q, (lo, hi) in enumerate(zip(wsp_edges[:-1], wsp_edges[1:]))]
    c_wr = cp(wr_hbm, wraw_s.at[0], 21)
    c_wi = cp(wi_hbm, wraw_s.at[1], 22)
    c_tw = cp(tw_hbm, tw_s, 23)
    c_mats = cp(mats_hbm.at[pl.ds(128, 160), :], mats_s.at[pl.ds(128, 160), :], 24)
    c_b = cp(b_hbm, b_s, 25)
    c_zero = cp(zero_hbm, zero_s, 10)
    c_mats2 = cp(mats_hbm.at[pl.ds(0, 128), :], mats_s.at[pl.ds(0, 128), :], 19)
    c_wout = cp(wout_hbm, wout_s, 26)
    out_cps = [cp(out_s.at[pl.ds(128 * t, 128), :], out_hbm.at[0, pl.ds(128 * t, 128), :], 27 + t)
               for t in range(16)]

    for c in [c_zero] + x_cps[0] + [c_gf, c_win2, c_win2b, c_win1] + x_cps[1] + x_cps[2] + x_cps[3] + [
            c_wr, c_wi, c_wout, c_b, c_small, c_wsp[0], c_mats, c_tw] + c_wsp[1:] + [c_mats2]:
        c.start()

    def lane_mask(n, kind="even"):
        ln = jax.lax.broadcasted_iota(jnp.int32, (n, 128), 1)
        if kind == "even":
            return (ln & 1) == 0
        if kind == "lo":
            return ln < 64
        return ((ln + 1) & 2) == 0

    row16 = jax.lax.broadcasted_iota(jnp.int32, (16, 512), 0)
    win_s[pl.ds(2 * HM + FH, 16), :] = jnp.where(row16 == 0, 1.0, 0.0).astype(BF16)
    win_s[pl.ds(FH, 16), :] = jnp.zeros((16, 512), BF16)

    c_zero.wait()
    z0 = zero_s[0]
    zero = jnp.full((8, 128), z0, jnp.int32).astype(U32)

    def dyn(ref):
        cnt[0] += 1
        return ref.at[z0 * (cnt[0] + 1)]

    xn_s, z1_s, aop_s, b1_s, wt_s = xn_f.at[z0], z1_f.at[z0], aop_f.at[z0], b1_f.at[z0], wt_f.at[z0]
    o_s, woT_s, b2_s = o_f.at[z0], woT_f.at[z0], b2_f.at[z0]
    st_s, ac_s = st_f.at[z0], ac_f.at[z0]
    b4_s, wsum_s, xs_s = b4_f.at[z0], wsum_f.at[z0], xs_f.at[z0]

    def mask0(dep):
        reps = dep.shape[-2] // 8
        z = zero if reps == 1 else jnp.concatenate([zero] * reps, axis=0)
        z = jnp.broadcast_to(z, dep.shape) if dep.ndim > 2 else z
        return pltpu.bitcast(dep, U32) & z

    def tie0(v, d):
        if v.dtype == U32:
            return v | d
        return pltpu.bitcast(pltpu.bitcast(v, U32) | d, F32)

    def tie(v, dep):
        return tie0(v, mask0(dep))

    def ctie(u, d, both=True):
        (re, sr), (im, si) = u
        return ((tie0(re, d), sr), (tie0(im, d) if both else im, si))

    def pick(rs, n):
        tot = sum(r.shape[0] // 8 for r in rs)
        out = []
        for u in range(n):
            g = (u * tot) // n
            for r in rs:
                m = r.shape[0] // 8
                if g < m:
                    out.append(r[8 * g:8 * g + 8, 0:128])
                    break
                g -= m
        return out

    US = {}

    def pre(i, e, deps):
        xu = dyn(xn_f)[pl.ds(256 * e + 64 * i, 64), :]
        if deps is not None:
            d = mask0(jnp.concatenate(deps, axis=0))
            xu = jnp.concatenate([xu[:, 0:128] | d, xu[:, 128:256] | d, xu[:, 256:]], axis=1)
        xf = _up(xu)
        x0, x1, x2, x3 = [xf[:, 128 * k:128 * (k + 1)] for k in range(4)]
        s02, s13 = x0 + x2, x1 + x3
        p, q = x0 - x2, x1 - x3
        lo = lane_mask(128, "lo")
        sv = jnp.where(lo, p, (p + q) * RH)
        rc = pltpu.roll(jnp.where(lo, q, (p - q) * RH), 64, 1)
        US[i, e] = (s02 + s13, s02 - s13, sv + rc, sv - rc)

    def ln1_block(i, e, deps):
        x = x_s[e, pl.ds(128 * i, 128), :].astype(F32)
        m = jnp.sum(x, axis=1, keepdims=True) * (1.0 / D)
        xc = x - m
        v = jnp.sum(xc * xc, axis=1, keepdims=True) * (1.0 / D)
        rstd = _rsqrt(jnp.broadcast_to(v + EPS, (128, 128)))
        if deps is not None:
            rstd = tie(rstd, jnp.concatenate(deps, axis=0))
        xn = xc * jnp.concatenate([rstd] * 4, axis=1)
        xn_s[pl.ds(256 * e + 64 * i, 64), :] = _pack(xn)
        return xn

    def ln1(i, es, deps=None):
        for n, e in enumerate(es):
            ln1_block(i, e, None if deps is None else deps[16 * n:16 * n + 16])

    def ln1_pair(i, e, deps):
        xa = ln1_block(i, e, [deps[4 * (k // 2) + k % 2] for k in range(16)])
        xb = ln1_block(i, e + 2, [deps[4 * (k // 2) + 2 + k % 2] for k in range(16)])
        b11, b21, b12, b22 = xa[:, 0:256], xa[:, 256:], xb[:, 0:256], xb[:, 256:]
        for k, v in enumerate([b11 + b22, b12 - b22, b21 - b11, b11 + b12, b21 + b22]):
            xs_s[4 * e + i, :, pl.ds(256 * k, 256)] = _pack(v)

    def wsum(deps):
        d = jnp.concatenate([mask0(jnp.concatenate([v for v in deps[c::2] for _ in range(2)], axis=0))
                             for c in range(2)], axis=1)
        blk = lambda r, c: win_s[pl.ds(2 * HM * r, 2 * HM), pl.ds(256 * c, 256)].astype(F32)
        a11, a22, a12, a21 = tie0(blk(0, 0), d), tie0(blk(1, 1), d), blk(0, 1), blk(1, 0)
        for k, v in enumerate([a11 + a22, a21 + a22, a11, a22, a11 + a12, a21 - a11, a12 - a22]):
            wsum_s[:, pl.ds(256 * k, 256)] = _pack(v)

    def dfwd(i):
        us = [jnp.concatenate([US[i, e][k][16 * r:16 * r + 16] for r in range(8) for e in range(4)],
                              axis=0).astype(BF16) for k in range(4)]
        gf = _unpack(gf_s[...])
        o0, o2, op, om = [jnp.dot(us[k], gf[:, 128 * k:128 * (k + 1)], preferred_element_type=F32)
                          for k in range(4)]
        ev, mp = lane_mask(512), lane_mask(512, "mp")
        re = jnp.stack([jnp.where(ev, o0, o2), jnp.where(mp, op, om)])
        im = jnp.stack([pltpu.roll(jnp.where(ev, o2, o0), 1, 1), pltpu.roll(jnp.where(mp, om, op), 2, 1)])
        re = re.reshape(2, 8, 4, 2, 8, 128)
        im = im.reshape(2, 8, 4, 2, 8, 128)
        outs = _dft([_cx(re[:, :, e], im[:, :, e]) for e in range(4)], 1)
        for ke in range(4):
            for ri in range(2):
                b1_s[ri, :, pl.ds(2 * i, 2), ke] = _val(outs[ke][ri]).reshape(2, 2, 8, 8, 128)

    AL = {}

    def zt2(sig):
        lhs = dyn(win_f)[pl.ds(2 * HM, 2 * HM), :]
        rhs = _unpack(xn_s[pl.ds(64 * sig, 64), :])
        r = jax.lax.dot_general(lhs, rhs, NT, preferred_element_type=F32)
        return r, z2_post(sig, r)

    def z2_post(sig, r, top=None):
        n = r.shape[0] - 16
        z2 = _gelu2(r[0:n]) if top is None else jnp.concatenate([top, _gelu2(r[0:n])], axis=0)
        a2_s[pl.ds(sig, 1), :] = r[n:n + 1]
        mu = jnp.sum(z2, axis=0, keepdims=True) * (1.0 / FH)
        ms = jnp.sum(z2 * z2, axis=0, keepdims=True) * (1.0 / FH)
        var = jnp.maximum(ms - mu * mu, 0.0)
        rstd = _rsqrt(jnp.broadcast_to(var + 4.0 * EPS, (8, 128)))
        mr = jnp.broadcast_to(mu, (8, 128)) * rstd

        def norm(deps=None):
            for q in range(11):
                rq = rstd if deps is None else tie(rstd, deps[q])
                rq, mq = jnp.concatenate([rq] * 4, axis=0), jnp.concatenate([mr] * 4, axis=0)
                top = z2[32 * q:32 * q + 32] * rq - mq
                nb = 32 if q < 10 else 16
                bot = z2[HM + 32 * q:HM + 32 * q + nb] * rq[0:nb] - mq[0:nb]
                if nb < 32:
                    bot = jnp.concatenate([bot, jnp.zeros((16, 128), F32)], axis=0)
                if sig < 8:
                    AL[sig, q] = (top, bot)
                else:
                    a11, a21 = AL.pop((sig - 8, q))
                    ops = [a11 + bot, a21 + bot, a11, bot, a11 + top, a21 - a11, top - bot, bot]
                    aop_s[pl.ds(16 * q, 16), pl.ds(1024 * (sig - 8), 1024)] = _pack(jnp.concatenate(ops, axis=1))
        return norm

    def zt1(sig):
        lhs = dyn(win_f)[pl.ds(0, FH), :]
        rhs = _unpack(xn_s[pl.ds(64 * sig, 64), :])
        r = jax.lax.dot_general(lhs, rhs, NT, preferred_element_type=F32)
        z1_s[sig] = _gelu2(r)
        return r

    pend = []

    def run(piece, sig):
        out = piece(sig)
        r = out[0] if piece is zt2 else out
        while pend:
            pend.pop()(pick([r], 11))
        if piece is zt2:
            pend.append(out[1])
        return r

    def zpair(sig, hook=None):
        rs = []

        def prod(k, rows=(0, HM)):
            lo, n = rows
            a = dyn(wsum_f)[pl.ds(lo, n), pl.ds(256 * k, 256)]
            if k == 1:
                b = xn_s[pl.ds(64 * sig, 64), pl.ds(0, 256)]
            elif k == 4:
                b = xn_s[pl.ds(64 * (sig + 8), 64), pl.ds(256, 256)]
            else:
                b = xs_s[sig, :, pl.ds(256 * {0: 0, 2: 1, 3: 2, 5: 3, 6: 4}[k], 256)]
            r = jax.lax.dot_general(_unpack(a), _unpack(b), NT, preferred_element_type=F32)
            rs.append(r)
            return r

        def release(r):
            while pend:
                pend.pop()(pick([r], 11))

        m2, m4 = prod(1), prod(3)
        release(m4)
        pend.append(z2_post(sig, m2 + m4))
        if sig == 7:
            m3, m6 = prod(2), prod(5)
            release(m6)
            t22 = m3 - m2 + m6
            m1, m5 = prod(0), prod(4)
            pend.append(z2_post(sig + 8, t22 + m1))
            z1_s[sig + 8] = _gelu2((m3 + m5)[0:FH])
            t11 = m4 - m5 + m1
            hook(rs)
            m7 = jnp.concatenate([prod(6, (0, HM // 2)), prod(6, (HM // 2, HM // 2))], axis=0)
            release(m7)
            z1_s[sig] = _gelu2((t11 + m7)[0:FH])
            return None
        m3, m5 = prod(2), prod(4)
        release(m5)
        z1_s[sig + 8] = _gelu2((m3 + m5)[0:FH])
        t11, t22 = m4 - m5, m3 - m2
        m1, m7 = prod(0), prod(6)
        z1_s[sig] = _gelu2((t11 + m1 + m7)[0:FH])
        t22 = t22 + m1
        m6 = prod(5)
        pend.append(z2_post(sig + 8, t22 + m6))
        return [m4, m5, m7, m6]

    def zhalf(sig, lo):
        return jax.lax.dot_general(dyn(win_f)[pl.ds(2 * HM + lo, HM), :], _unpack(xn_s[pl.ds(64 * sig, 64), :]),
                                   NT, preferred_element_type=F32)

    x_cps[0][0].wait()
    ln1(0, (0, 1))
    pre(0, 0, None)
    pre(0, 1, None)
    x_cps[0][1].wait()
    c_gf.wait()
    ln1(0, (2, 3))
    pre(0, 2, None)
    pre(0, 3, None)
    dfwd(0)
    c_win2.wait()
    tops = [_gelu2(zhalf(4 * e, 0)) for e in range(4)]
    c_win2b.wait()
    for e in range(4):
        r = zhalf(4 * e, HM)
        while pend:
            pend.pop()(pick([r], 11))
        pend.append(z2_post(4 * e, r, tops[e]))
    c_win1.wait()
    x_cps[1][0].wait()
    x_cps[1][1].wait()

    def both(sigs):
        return [run(zt, sig) for sig in sigs for zt in (zt2, zt1)]

    def pres(i, rs):
        deps = pick(rs, 32)
        for e in range(4):
            pre(i, e, deps[8 * e:8 * e + 8])

    rs = [run(zt1, 4 * e) for e in range(4)]
    ln1(1, (0, 2), pick(rs[:3], 32))
    rs = rs[3:] + both((1,))
    wsum(pick(rs[:2] + [rs[2][0:344]], 88))
    x_cps[1][2].wait()
    x_cps[1][3].wait()
    for i in (2, 3):
        for c in x_cps[i]:
            c.wait()
    rs = both((9,))
    ln1_pair(1, 1, pick([rs[0], rs[1][0:400]], 32))
    rs = zpair(5)
    ln1_pair(2, 0, pick(rs[:3], 32))
    rs = zpair(2)
    ln1_pair(2, 1, pick(rs[:3], 32))
    rs = zpair(6)
    ln1_pair(3, 0, pick(rs[:3], 32))
    rs = zpair(3)
    ln1_pair(3, 1, pick(rs[:2], 32))
    pres(1, rs[2:])
    zpair(7, hook=lambda rs: (pres(2, rs[1:2]), pres(3, rs[3:4]), dfwd(1), dfwd(2), dfwd(3)))

    for c in (c_wr, c_wi, c_wout, c_b, c_small, c_wsp[0], c_mats):
        c.wait()

    links = []

    def wprep(deps):
        row = jax.lax.broadcasted_iota(jnp.int32, (16, 128), 0)
        for p in range(2):
            for kb in range(16):
                cols = pl.ds(128 * kb, 128)
                top = wraw_s[p, pl.ds(0, 16), cols].astype(F32)
                ny = wraw_s[p, pl.ds(256, 1), cols].astype(F32)
                top = jnp.where(row == 0, jnp.broadcast_to(ny, (16, 128)), top)
                d = deps[16 * p + kb]
                blk = jnp.concatenate([tie(_pack(top), d),
                                       pltpu.bitcast(wraw_s[p, pl.ds(16, 240), cols], U32)], axis=0)
                bt = blk.T
                wt_s[p, pl.ds(128 * kb, 128), :] = bt
                links.append(bt[120:128])

    def woprep(deps):
        w = pltpu.bitcast(wout_s[...], U32)
        cols = []
        for cb in range(4):
            rows = []
            for rb in range(6):
                blk = w[64 * rb:min(64 * rb + 64, FH // 2), 128 * cb:128 * cb + 128]
                rows += [tie(blk[0:8], deps[6 * cb + rb]), blk[8:]]
            cols.append(jnp.concatenate(rows, axis=0))
        woT_s[...] = pltpu.bitcast(_unpack(jnp.concatenate(cols, axis=1)).T, U32)

    def compact():
        mats = _unpack(mats_s[pl.ds(128, 160), :])
        mf, mi = mats[0:128], mats[128:256]
        f16, i16 = mats[256:288, 0:16], mats[288:304, 0:32]
        tc, ts = small_s[pl.ds(0, 16), :], small_s[pl.ds(16, 16), :]
        u = jnp.dot(f16, a2_s[...].astype(BF16), preferred_element_type=F32)
        ur, ui = u[0:16], u[16:32]
        ur, ui = ur * tc + ui * ts, ui * tc - ur * ts
        yield None
        r = jnp.dot(jnp.concatenate([ur, ui], axis=0).astype(BF16), mf, preferred_element_type=F32)
        pr, pi = r[0:16, 0:128] + r[16:32, 128:256], r[16:32, 0:128] - r[0:16, 128:256]
        blk = jax.lax.broadcasted_iota(jnp.int32, (16, 128), 1) // 16
        w0 = []
        for p in range(2):
            wn = jnp.concatenate([wraw_s[p, pl.ds(0, 8), pl.ds(128 * be, 128)].astype(F32)[0:1]
                                  for be in range(16)], axis=0)
            tf = jnp.concatenate([wn] * 8, axis=0).T
            acc = tf[0:16]
            for ka in range(1, 8):
                acc = jnp.where(blk == ka, tf[16 * ka:16 * ka + 16], acc)
            w0.append(acc)
        yr, yi = pr * w0[0] - pi * w0[1], pr * w0[1] + pi * w0[0]
        yield None
        r = jnp.dot(jnp.concatenate([yr, yi], axis=0).astype(BF16), mi, preferred_element_type=F32)
        vr, vi = r[0:16, 0:128] - r[16:32, 128:256], r[16:32, 0:128] + r[0:16, 128:256]
        vr, vi = vr * tc - vi * ts, vi * tc + vr * ts
        yield None
        ap = jnp.dot(i16, jnp.concatenate([vr, vi], axis=0).astype(BF16), preferred_element_type=F32)
        apT = jnp.concatenate([ap] * 8, axis=0).T
        for s2 in range(16):
            ac_s[pl.ds(128 * s2, 128), :] = jnp.broadcast_to(apT[:, s2:s2 + 1], (128, 128))
        yield None

    def split(deps, shape):
        return [mask0(jnp.concatenate(deps[k::2], axis=0).reshape(shape)) for k in range(2)]

    def tied(ins, d, full=False):
        if full:
            return [ctie(u, d[1 - q % 2]) for q, u in enumerate(ins)]
        ins[1], ins[0] = ctie(ins[1], d[0]), ctie(ins[0], d[1])
        return ins

    def cstack(us, axis):
        return _cx(*[jnp.stack([_val(u[ri]) for u in us], axis=axis) for ri in range(2)])

    V = {}

    def p2(deps):
        for ke in range(4):
            for b in range(8):
                n = 4 * (8 * ke + b)
                ins = tied([_cx(b1_s[0, :, a, ke, b], b1_s[1, :, a, ke, b]) for a in range(8)],
                           split(deps[n:n + 4], (2, 8, 128)))
                outs = _dft([_crot(ins[a], (8 * a + b) * ke, 256) for a in range(8)], 1)
                for ka in range(8):
                    V[ka, ke, b] = outs[ka]

    def p3(deps):
        for ka in range(8):
            ins = tied([cstack([V[ka, ke, b] for ke in range(4)], 1) for b in range(8)],
                       split([deps[2 * (16 * ke + 2 * ka + t) + k] for t in range(2) for ke in range(4)
                              for k in range(2)], (2, 4, 8, 128)), True)
            outs = _dft([_crot(ins[b], b * ka, 64) for b in range(8)], 1)
            for kb in range(8):
                for ri in range(2):
                    b2_s[ri, :, pl.ds(256 * kb + 32 * ka, 32), :] = _val(outs[kb][ri]).reshape(2, 32, 128)

    def mid(t, deps):
        d = [mask0(jnp.concatenate(deps[k::5], axis=0)) for k in range(5)]
        twa, twb, wt = dyn(tw_f), dyn(tw_f), dyn(wt_f)
        ins = []
        for c in range(8):
            u = _cx(b2_s[0, t, pl.ds(c, 256, stride=8), :], b2_s[1, t, pl.ds(c, 256, stride=8), :])
            if c < 2:
                u = ctie(u, d[1 - c], both=(c == 0))
            ins.append(u if c == 0 else _cmul_vec(u, twa[2 * c - 2], twa[2 * c - 1], False))
        outs = _dft(ins, 1)
        sel = [d[3 - k] | jnp.uint32(16 if t == 0 else 0xFFFF0000) for k in range(2)]
        ys = []
        for kc in range(8):
            wr, wi = wt[0, pl.ds(256 * kc, 256), :], wt[1, pl.ds(256 * kc, 256), :]
            if t == 0:
                wr, wi = wr << sel[kc % 2], wi << sel[kc % 2]
            else:
                wr, wi = wr & sel[kc % 2], wi & sel[kc % 2]
            ys.append(_cmul_vec(outs[kc], pltpu.bitcast(wr, F32), pltpu.bitcast(wi, F32), True))
        outs = _dft(ys, -1)
        for c in range(8):
            o = outs[c] if c == 0 else _cmul_vec(outs[c], tie0(twb[2 * c - 2], d[4]), twb[2 * c - 1], True)
            b4_s[0, t, pl.ds(c, 256, stride=8), :] = _val(o[0])
            b4_s[1, t, pl.ds(c, 256, stride=8), :] = _val(o[1])

    def p3i(deps):
        ins = tied([_cx(b4_s[0, :, pl.ds(256 * kb, 256), :], b4_s[1, :, pl.ds(256 * kb, 256), :])
                    for kb in range(8)], split(deps, (2, 256, 128)))
        outs = _dft(ins, -1)
        for b in range(8):
            (re, sr), (im, si) = outs[b]
            re, im = re.reshape(2, 8, 4, 8, 128), im.reshape(2, 8, 4, 8, 128)
            for ka in range(8):
                V[ka, b] = ((re[:, ka], sr), (im[:, ka], si))

    def p2i(deps):
        for b in range(8):
            ins = tied([V[ka, b] for ka in range(8)],
                       split([deps[2 * (32 * t + 4 * b + ke) + k] for t in range(2) for ke in range(4)
                              for k in range(2)], (2, 4, 8, 128)), True)
            outs = _dft([_crot(ins[ka], -b * ka, 64) for ka in range(8)], -1)
            for a in range(8):
                (re, sr), (im, si) = outs[a]
                for ke in range(4):
                    V[a, ke, b] = ((re[:, ke], sr), (im[:, ke], si))

    def p1i(deps):
        ev, mp = lane_mask(16), lane_mask(16, "mp")
        l0 = jax.lax.broadcasted_iota(jnp.int32, (16, 128), 1) == 0
        for a in range(8):
            for bp in range(4):
                n = 4 * a + bp
                d = split([deps[2 * (32 * t + 8 * bp + a) + k] for t in range(2) for k in range(2)], (2, 8, 128))
                res = []
                for hh in range(2):
                    b = 2 * bp + hh
                    ins = [ctie(V[a, ke, b], d[hh]) for ke in range(4)]
                    res.append(_dft([_crot(ins[ke], -(8 * a + b) * ke, 256) for ke in range(4)], -1))
                r0 = 64 * a + 16 * bp
                for e in range(4):
                    re = jnp.concatenate([_val(res[0][e][0]), _val(res[1][e][0])], axis=1)
                    im = jnp.concatenate([_val(res[0][e][1]), _val(res[1][e][1])], axis=1)
                    col = ac_s[pl.ds(512 * e + r0, 16), :]
                    ri = pltpu.roll(jnp.where(l0, col, im[0]), 127, 1)
                    i0, i2 = jnp.where(ev, re[0], ri), jnp.where(ev, ri, re[0])
                    rb = pltpu.roll(im[1], 126, 1)
                    ip, in_ = jnp.where(mp, re[1], rb), jnp.where(mp, rb, re[1])
                    st_s[pl.ds(256 * e + r0 // 2, 8), :] = _pack(jnp.concatenate([i0, i2, ip, in_], axis=1))

    def gpair(j):
        rows = pl.ds(128 * j, 128)

        def prod(k):
            a = dyn(aop_f)
            held = list(links)
            del links[:]
            wv = dyn(wsp_f)
            blk = lambda q, u: wv[q[1], rows, pl.ds(1024 * q[0] + 512 * u, 512)]
            x, sg, y = {1: ((0, 0), 0, None), 4: ((1, 1), 0, None), 0: ((0, 0), 1, (1, 1)), 2: ((0, 1), -1, (1, 1)),
                        3: ((1, 0), -1, (0, 0)), 5: ((0, 0), 1, (0, 1)), 6: ((1, 0), 1, (1, 1))}[k]

            def rhs(u):
                if sg == 0:
                    return blk(x, u)
                p, q = blk(x, u).astype(F32), blk(y, u).astype(F32)
                return (p + q if sg > 0 else p - q).astype(BF16)
            nr = (FH - HM if k in (1, 5) else HM) // 2
            lhs = [jnp.concatenate([a[pl.ds(0, nr), pl.ds(1024 * c + 128 * k, 128)] for c in range(4 * u, 4 * u + 4)],
                                   axis=1) for u in range(2)]
            r = [jax.lax.dot_general(_unpack(lhs[0]), rhs(0), NT, preferred_element_type=F32)]
            for ev in events.get(NP[0] + 0.5, ()):
                ev()
            r.append(jax.lax.dot_general(_unpack(lhs[1]), rhs(1), NT, preferred_element_type=F32))
            n = NP[0]
            NP[0] += 1
            RS.extend([(n, r[0]), (n + 0.5, r[1])])
            r0 = r[0]
            if held:
                acc = held.pop()
                while held:
                    acc = acc | held.pop()
                r0 = jnp.concatenate([r0[0:240], tie0(r0[240:248], acc & zero), r0[248:]], axis=0)
            for ev in events.get(NP[0], ()):
                ev()
            return r0 + r[1]

        def gate_in(t, top, bot):
            g = jnp.concatenate([top, bot[0:FH - HM]], axis=0) + b_s[pl.ds(t, 1), :].astype(F32)
            H[t] = (z1_s[t] * g).astype(BF16)

        nb = FH - HM
        m2 = prod(1)
        m5 = prod(4)
        m4 = prod(3)
        c21, t11 = m2 + m4[0:nb], m4 - m5
        m1 = prod(0)
        t11, t22 = t11 + m1, m1[0:nb] - m2
        gate_in(j, t11 + prod(6), c21)
        m3 = prod(2)
        c12, t22 = m3 + m5, t22 + m3[0:nb]
        gate_in(j + 8, c12, t22 + prod(5))

    def bout(t, h):
        wo = dyn(woT_f)
        oT = jnp.concatenate([jnp.dot(_unpack(wo[pl.ds(128 * q, 128), :]), h, preferred_element_type=F32)
                              for q in range(2)], axis=0)
        RS.append((NP[0] - 0.25, oT))
        ho = 0.25 * oT
        gate = ho + ho * jnp.tanh(ho)
        gT = pltpu.bitcast(gate.astype(BF16).T, U32)
        o_s[pl.ds(64 * t, 64), :] = gT
        if t % 8 <= 4:
            links.extend([gT[56:64, 128 * q:128 * q + 128] for q in range(4)])
        return oT

    def final(t):
        gi = _unpack(mats_s[pl.ds(0, 128), :])
        z = _unpack(st_s[pl.ds(64 * t, 64), :])
        v0, v2, tp, tm = [jnp.dot(z[:, 128 * k:128 * (k + 1)],
                                  gi[128 * (k // 2):128 * (k // 2) + 128, 128 * (k % 2):128 * (k % 2) + 128],
                                  preferred_element_type=F32) for k in range(4)]
        sp, sm = v0 + v2, v0 - v2
        ss, df = tp + tm, tp - tm
        lo = lane_mask(128, "lo")
        rc = pltpu.roll(jnp.where(lo, df, ss), 64, 1)
        pp, qn = jnp.where(lo, ss, (rc - df) * RH), jnp.where(lo, rc, (rc + df) * RH)
        y = jnp.concatenate([sp + pp, sm - qn, sp - pp, sm + qn], axis=1)
        gate = _unpack(o_s[pl.ds(64 * t, 64), :]).astype(F32)
        x = x_s[t // 4, pl.ds(128 * (t % 4), 128), :].astype(F32)
        out_s[pl.ds(128 * t, 128), :] = (x + y * gate).astype(BF16)
        out_cps[t].start()

    RS, H, NP = [], {}, [0]
    cgen = compact()
    events = {}

    def at(n, fn):
        events.setdefault(n, []).append(fn)

    def span(fn, lo, hi, n, when=None):
        at(when or int(math.ceil(hi)), lambda: fn(pick([r for pos, r in RS if lo <= pos < hi], n)))

    def waits(*cps):
        return lambda: [c.wait() for c in cps]

    for j in range(1, 8):
        at(7 * j + 2, functools.partial(lambda t: bout(t, H[t]), j - 1))
        at(7 * j + 4, functools.partial(lambda t: bout(t, H[t]), j + 7))
    span(woprep, 2, 5, 24)
    span(p2, 0, 8, 128)
    span(wprep, 5, 13, 32)
    span(p3, 8.5, 16.5, 128, when=17)
    at(7, lambda: next(cgen))
    at(17, waits(c_wsp[1], c_tw))
    at(17, lambda: next(cgen))
    span(functools.partial(mid, 0), 17, 26, 160)
    at(22, lambda: next(cgen))
    span(functools.partial(mid, 1), 26, 34.5, 160, when=35)
    at(35, waits(c_wsp[2]))
    span(p3i, 35, 39, 128)
    span(p2i, 39.5, 44, 128)
    span(p1i, 44.5, 49.5, 128, when=50)
    at(50, waits(c_mats2))
    at(55, lambda: bout(7, H[7]))
    order = [0, 8, 1, 9, 2, 10, 3, 11, 4, 12, 5, 13, 6, 14]
    slots = [50, 50.5, 50.5, 51, 51.5, 52, 52, 52.5, 53, 53.5, 54, 54.5, 54.5, 55.5]
    for q in range(14):
        at(slots[q], functools.partial(final, order[q]))

    next(cgen)
    for j in range(8):
        gpair(j)
    final(7)
    bout(15, H[15])
    final(15)
    for c in out_cps:
        c.wait()


@jax.jit
def pallas_recurrent_scan__spectral_gfnet__mixer_gmlp__prompt_kernel(
    A_x: jax.Array,
    A_w_r: jax.Array,
    A_w_i: jax.Array,
    B_x: jax.Array,
    B_w_in: jax.Array,
    B_w_sp: jax.Array,
    B_b_sp: jax.Array,
    B_w_out: jax.Array,
):
    gf, mats, tw, small = _constants()
    args = (A_x.reshape(4, 512, 512), A_w_r.T, A_w_i.T, B_w_in.T, B_w_sp.reshape(2, 1024, 2048), B_b_sp.reshape(16, 128), B_w_out,
            jnp.asarray(gf), jnp.asarray(mats), jnp.asarray(tw), jnp.asarray(small),
            jnp.asarray((np.arange(128) ** 2 % 7).astype(np.int32)))
    vm = pltpu.VMEM
    scratch = [
        vm((4, 512, 512), BF16),
        vm((1, 1024, 512), U32),
        vm((1, 4 * HM, 512), BF16),
        vm((1, HM, 1792), U32),
        vm((1, 8, 64, 1280), U32),
        vm((1, 16, FH, 128), F32),
        vm((1, HM // 2, 8192), U32),
        vm((1, 2, 1024, 2048), BF16),
        vm((1, 2, 2, 8, 4, 8, 8, 128), F32),
        vm((1, 2, 2, 2048, 128), F32),
        vm((1, 2, 2, 2048, 128), F32),
        vm((2, DF, 2048), BF16),
        vm((1, 2, 2048, 128), U32),
        vm((64, 512), U32),
        vm((288, 256), U32),
        vm((1, 14, 256, 128), F32),
        vm((40, 128), F32),
        vm((16, 128), BF16),
        vm((FH, 512), BF16),
        vm((1, 256, FH), U32),
        vm((16, 128), F32),
        vm((1, 2048, 128), F32),
        vm((1, 1024, 512), U32),
        vm((1, 1024, 512), U32),
        vm((2048, 512), BF16),
        pltpu.SMEM((128,), jnp.int32),
        pltpu.SemaphoreType.DMA((51,)),
    ]
    return pl.pallas_call(
        _kernel,
        out_shape=jax.ShapeDtypeStruct((1, S, D), BF16),
        in_specs=[pl.BlockSpec(memory_space=pl.ANY)] * len(args),
        out_specs=pl.BlockSpec(memory_space=pl.ANY),
        scratch_shapes=scratch,
        compiler_params=pltpu.CompilerParams(vmem_limit_bytes=100 * 1024 * 1024,
                                             disable_semaphore_checks=True, disable_bounds_checks=True),
    )(*args)
```
